```python
import jax
import jax.numpy as jnp

def _softmax(x, axis=-1):
    return jax.nn.softmax(x, axis=axis)
def _gelu(x):
    return jax.nn.gelu(x, approximate=True)
def _silu(x):
    return jax.nn.silu(x)
def _sigmoid(x):
    return jax.nn.sigmoid(x)
def _layernorm(x, axis=-1, eps=1e-5):
    m = jnp.mean(x, axis=axis, keepdims=True)
    v = jnp.var(x, axis=axis, keepdims=True)
    return (x - m) / jnp.sqrt(v + eps)
def _scatter_add(tgt, idx, src, axis=0):
    return tgt.at[idx].add(src)
def _segment_sum(src, seg, n):
    return jax.ops.segment_sum(src, seg, n)
class _Rng:
    def __init__(self, key):
        self._k = key
    def _next(self):
        self._k, sub = jax.random.split(self._k)
        return sub
    def normal(self, shape):
        return jax.random.normal(self._next(), shape, dtype=jnp.bfloat16)
    def randint(self, lo, hi, shape):
        return jax.random.randint(self._next(), shape, lo, hi, dtype=jnp.int32)
    def uniform(self, shape, lo=0.0, hi=1.0):
        return jax.random.uniform(self._next(), shape, jnp.bfloat16, lo, hi)
    def permutation(self, n):
        return jax.random.permutation(self._next(), n)


kernel_name = 'interleave_layers__sliding_block_cached__dense_activation_gelu__decode'

def _fwd_setup_inputs():
    _rng = _Rng(jax.random.key(int.from_bytes(__import__("os").urandom(4), "little")))
    _w = (lambda a: (lambda t: t.astype(jnp.bfloat16) if jnp.issubdtype(t.dtype, jnp.floating) else t)(jnp.asarray(a)))
    def _A_setup():
        B, Sq, D = 2, 1, 512
        Hq, Hkv, Sk, Dh = 32, 8, 32768, 128
        assert Hq % Hkv == 0, (Hq, Hkv)
        return {
            "x": _w((lambda *s: _rng.normal(s) * 0.05)(B, Sq, D)),
            "k_cache": _w((lambda *s: _rng.normal(s) * 0.05)(B, Hkv, Sk, Dh)),
            "v_cache": _w((lambda *s: _rng.normal(s) * 0.05)(B, Hkv, Sk, Dh)),
            "wq": _w((lambda *s: _rng.normal(s) * 0.05)(D, Hq * Dh) * (D ** -0.5)),
            "wo": _w((lambda *s: _rng.normal(s) * 0.05)(Hq * Dh, D) * ((Hq * Dh) ** -0.5)),
        }
    _A_in = _A_setup()

    def _B_setup():
        B, S, D, F = 2, 1, 512, 1792
        return {
            "x": _w((lambda *s: _rng.normal(s) * 0.05)(B, S, D)),
            "w1": _w((lambda *s: _rng.normal(s) * 0.05)(D, F) * (D ** -0.5)),
            "b1": _w((lambda *s: _rng.normal(s) * 0.05)(F) * 0.01),
            "w2": _w((lambda *s: _rng.normal(s) * 0.05)(F, D) * (F ** -0.5)),
            "b2": _w((lambda *s: _rng.normal(s) * 0.05)(D) * 0.01),
        }
    _B_in = _B_setup()

    return {
        "A_x": _A_in["x"],
        "A_k_cache": _A_in["k_cache"],
        "A_v_cache": _A_in["v_cache"],
        "A_wq": _A_in["wq"],
        "A_wo": _A_in["wo"],
        "B_x": _B_in["x"],
        "B_w1": _B_in["w1"],
        "B_b1": _B_in["b1"],
        "B_w2": _B_in["w2"],
        "B_b2": _B_in["b2"],
    }

def _fwd_reference(A_x, A_k_cache, A_v_cache, A_wq, A_wo, B_x, B_w1, B_b1, B_w2, B_b2):
    def _A_ref(x, k_cache, v_cache, wq, wo):
        B, Sq, D = x.shape
        Hq, Dh = 32, 128
        Hkv, Sk = k_cache.shape[1], k_cache.shape[2]
        W = min(4096, max(256, Sk // 4))
        rep = Hq // Hkv
        q = (lambda x, *d: x.transpose(*d))((x @ wq).reshape(B, Sq, Hq, Dh), 0, 2, 1, 3)
        k = jnp.repeat(k_cache[:, :, Sk - W:, :], rep, axis=1)
        v = jnp.repeat(v_cache[:, :, Sk - W:, :], rep, axis=1)
        scores = jnp.einsum("bhqd,bhkd->bhqk", q, k) * (Dh ** -0.5)
        p = _softmax(scores, axis=-1)
        o = jnp.einsum("bhqk,bhkd->bhqd", p, v)
        return (lambda x, *d: x.transpose(*d))(o, 0, 2, 1, 3).reshape(B, Sq, Hq * Dh) @ wo

    def _B_ref(x, w1, b1, w2, b2):
        h = jnp.einsum("bsd,df->bsf", x, w1) + b1
        h = _gelu(h)
        return jnp.einsum("bsf,fd->bsd", h, w2) + b2

    x = A_x
    x = x + _A_ref(_layernorm(x, axis=-1), A_k_cache, A_v_cache, A_wq, A_wo)
    x = x + _B_ref(_layernorm(x, axis=-1), B_w1, B_b1, B_w2, B_b2)
    x = x + _A_ref(_layernorm(x, axis=-1), A_k_cache, A_v_cache, A_wq, A_wo)
    x = x + _B_ref(_layernorm(x, axis=-1), B_w1, B_b1, B_w2, B_b2)
    return x


def setup_inputs():
    _inp = _fwd_setup_inputs()
    _gk = jax.random.fold_in(jax.random.key(int.from_bytes(__import__("os").urandom(4), "little")), 2**31 - 1)
    _shapes = [[2, 1, 512]]
    _dtypes = ['bfloat16']
    _gks = jax.random.split(_gk, len(_shapes))
    _gs = [jax.random.normal(k, s, dtype=jnp.dtype(d)) * 0.05 for k, s, d in zip(_gks, _shapes, _dtypes)]
    _inp["grad_out"] = _gs[0]
    return _inp

def reference(A_x, A_k_cache, A_v_cache, A_wq, A_wo, B_w1, B_b1, B_w2, B_b2, B_x, grad_out):
    _const = dict(B_x=B_x)
    def _f(*_d):
        return _fwd_reference(**{'A_x': _d[0], 'A_k_cache': _d[1], 'A_v_cache': _d[2], 'A_wq': _d[3], 'A_wo': _d[4], 'B_w1': _d[5], 'B_b1': _d[6], 'B_w2': _d[7], 'B_b2': _d[8], **_const})
    _out, _vjp = jax.vjp(_f, A_x, A_k_cache, A_v_cache, A_wq, A_wo, B_w1, B_b1, B_w2, B_b2)
    _grads = _vjp(grad_out)
    _out0 = jnp.asarray(_out)
    return (_out0, *[jnp.asarray(_g) for _g in _grads])
```

```python
import math

import jax
import jax.numpy as jnp
from jax import lax
import jax.experimental.pallas as pl
import jax.experimental.pallas.tpu as pltpu

NB, DM, HQ, HKV, SK, DH, FF = 2, 512, 32, 8, 32768, 128, 1792
WIN = min(4096, max(256, SK // 4))
REP = HQ // HKV
Z0 = SK - WIN
EPS = 1e-5
SCALE = DH ** -0.5
GELU_C = math.sqrt(2.0 / math.pi)
GELU_A = 0.044715

NR = NB * HKV
NSEG = SK // WIN
ZR = 128
NJ = WIN // ZR
RG = 4
ZPI = 16
ZB = 16

f32 = jnp.float32
bf16 = jnp.bfloat16


def _nn(a, b):
    return lax.dot_general(a, b, (((1,), (0,)), ((), ())), preferred_element_type=f32)


def _nt(a, b):
    return lax.dot_general(a, b, (((1,), (1,)), ((), ())), preferred_element_type=f32)


def _tn(a, b):
    return lax.dot_general(a, b, (((0,), (0,)), ((), ())), preferred_element_type=f32)


def _rows(shape):
    return lax.broadcasted_iota(jnp.int32, shape, 0)


def _ln_fwd(x):
    m = jnp.mean(x, axis=-1, keepdims=True)
    xc = x - m
    v = jnp.mean(xc * xc, axis=-1, keepdims=True)
    rs = lax.rsqrt(v + EPS)
    return xc * rs, rs


def _ln_bwd(dy, y, rs):
    return rs * (dy - jnp.mean(dy, axis=-1, keepdims=True)
                 - y * jnp.mean(dy * y, axis=-1, keepdims=True))


def _group_sum(a):
    lo = _rows(a.shape) < 4
    s0 = jnp.sum(jnp.where(lo, a, 0.0), axis=0, keepdims=True)
    s1 = jnp.sum(jnp.where(lo, 0.0, a), axis=0, keepdims=True)
    return jnp.where(lo, s0, s1)


def _kernel(x_hbm, g_hbm, b1_hbm, b2_hbm,
            kc_hbm, vc_hbm, wq_hbm, wo_hbm, w1_hbm, w2_hbm,
            out_hbm, dx_hbm, db1_hbm, db2_hbm,
            dk_hbm, dv_hbm, dwq_hbm, dwo_hbm, dw1_hbm, dw2_hbm,
            x_ref, g_ref, b1_ref, b2_ref, out_ref, dx_ref, db1_ref, db2_ref,
            k_buf, v_buf, wq_buf, wo_buf, w1_buf, w2_buf, zbuf,
            dwq_buf, dwo_buf, dw1_buf, dw2_buf,
            q_scr, o_scr, do_scr, dq_scr, p_scr, ds_scr, full_scr,
            kv_sem, w_sem, z_sem, o_sem, wo_sem, s_sem, so_sem):
    def kv_in(i, c):
        r = i // NJ
        r0 = pl.multiple_of((i % NJ) * ZR, ZR)
        b = r // HKV
        kv = r % HKV
        pltpu.make_async_copy(kc_hbm.at[b, kv, pl.ds(Z0 + r0, ZR), :], k_buf.at[r, pl.ds(r0, ZR), :],
                              kv_sem.at[0]).start(priority=0)
        pltpu.make_async_copy(vc_hbm.at[b, kv, pl.ds(Z0 + r0, ZR), :], v_buf.at[r, pl.ds(r0, ZR), :],
                              kv_sem.at[1]).start(priority=1)
        return c

    def w_chunk(i, which, srcs, dsts, sem):
        def go(n, idx, prio):
            pltpu.make_async_copy(srcs[n].at[idx], dsts[n].at[idx], sem.at[n]).start(priority=prio)
        if 0 in which:
            go(0, (pl.ds(pl.multiple_of((i // 4) * 16, 16), 16),
                   pl.ds(pl.multiple_of((i % 4) * 1024, 1024), 1024)), 0)
        if 1 in which:
            go(1, (pl.ds(pl.multiple_of(i * 32, 32), 32), slice(None)), 1)
        if 2 in which:
            go(2, (pl.ds(pl.multiple_of((i // 2) * 16, 16), 16),
                   pl.ds(pl.multiple_of((i % 2) * 896, 128), 896)), 0)
        if 3 in which:
            go(3, (pl.ds(pl.multiple_of(i * 32, 32), 32), slice(None)), 1)

    w_ranges = ((0, 56, (0, 1, 2, 3)), (56, 64, (0, 1, 2)), (64, 128, (0, 1)))
    w_hbm = (wq_hbm, wo_hbm, w1_hbm, w2_hbm)
    w_buf = (wq_buf, wo_buf, w1_buf, w2_buf)
    dw_buf = (dwq_buf, dwo_buf, dw1_buf, dw2_buf)
    dw_hbm = (dwq_hbm, dwo_hbm, dw1_hbm, dw2_hbm)

    s_in = [pltpu.make_async_copy(s, d, s_sem.at[i]) for i, (s, d) in enumerate(
        ((x_hbm, x_ref), (g_hbm, g_ref), (b1_hbm, b1_ref), (b2_hbm, b2_ref)))]
    s_out = [pltpu.make_async_copy(s, d, so_sem.at[i]) for i, (s, d) in enumerate(
        ((out_ref, out_hbm), (dx_ref, dx_hbm), (db1_ref, db1_hbm), (db2_ref, db2_hbm)))]

    NZ = (NR // RG) * (NSEG - 1) * NJ

    def z_issue(i, c):
        g = i // ((NSEG - 1) * NJ)
        rem = i % ((NSEG - 1) * NJ)
        sg = rem // NJ
        r0 = pl.multiple_of((rem % NJ) * ZR, ZR)
        pltpu.make_async_copy(zbuf, dk_hbm.at[pl.ds(g * RG, RG), sg, pl.ds(r0, ZR), :],
                              z_sem.at[0]).start(priority=0)
        pltpu.make_async_copy(zbuf, dv_hbm.at[pl.ds(g * RG, RG), sg, pl.ds(r0, ZR), :],
                              z_sem.at[1]).start(priority=1)
        return c

    zc = [0]

    def z_batch(n):
        lax.fori_loop(zc[0], zc[0] + n, z_issue, 0)
        zc[0] += n

    def z_in_loop(kv):
        base = zc[0] + kv * ZPI
        lax.fori_loop(base, base + ZPI, z_issue, 0)

    def win_out(i, c):
        g = (i // NJ) * RG
        r0 = pl.multiple_of((i % NJ) * ZR, ZR)
        pltpu.make_async_copy(k_buf.at[pl.ds(g, RG), pl.ds(r0, ZR), :],
                              dk_hbm.at[pl.ds(g, RG), NSEG - 1, pl.ds(r0, ZR), :],
                              o_sem.at[0]).start(priority=0)
        pltpu.make_async_copy(v_buf.at[pl.ds(g, RG), pl.ds(r0, ZR), :],
                              dv_hbm.at[pl.ds(g, RG), NSEG - 1, pl.ds(r0, ZR), :],
                              o_sem.at[1]).start(priority=1)
        return c

    for c in s_in:
        c.start()
    for lo, hi, which in w_ranges:
        def w_in(i, c, which=which):
            w_chunk(i, which, w_hbm, w_buf, w_sem)
            return c
        lax.fori_loop(lo, hi, w_in, 0)
    zbuf[...] = jnp.zeros(zbuf.shape, zbuf.dtype)
    lax.fori_loop(0, NR * NJ, kv_in, 0)
    z_batch(16)
    for i, buf in enumerate(w_buf):
        pltpu.make_async_copy(buf, buf, w_sem.at[i]).wait()
    pltpu.make_async_copy(k_buf, k_buf, kv_sem.at[0]).wait()
    pltpu.make_async_copy(v_buf, v_buf, kv_sem.at[1]).wait()

    z_batch(24)

    lo_w = _rows((8, WIN)) < 4
    lo_d = _rows((8, DH)) < 4
    rr_d = _rows((8, DH)) % REP

    def split_heads(full, dst, l):
        for kv in range(HKV):
            acc = None
            for r in range(REP):
                h = kv * REP + r
                blk = jnp.where(rr_d == r, full[:, h * DH:(h + 1) * DH], 0.0)
                acc = blk if acc is None else acc + blk
            dst[l, kv] = acc

    def merge_heads(src, l, slot):
        for kv in range(HKV):
            g = src[l, kv]
            for r in range(REP):
                h = kv * REP + r
                full_scr[slot, :, h * DH:(h + 1) * DH] = jnp.where(rr_d == r, g, 0.0)

    def attn_fwd(l, nb):
        split_heads(_nn(nb, wq_buf[...]), q_scr, l)

        def body(kv, c):
            z_in_loop(kv)
            qg = q_scr[l, kv].astype(bf16)
            s = jnp.where(lo_w, _nt(qg, k_buf[kv]), _nt(qg, k_buf[HKV + kv])) * SCALE
            m = jnp.max(s, axis=-1, keepdims=True)
            e = jnp.exp(s - m)
            p = e / jnp.sum(e, axis=-1, keepdims=True)
            p_scr[l, kv] = p
            pb = p.astype(bf16)
            o_scr[l, kv] = jnp.where(lo_d, _nn(pb, v_buf[kv]), _nn(pb, v_buf[HKV + kv]))
            return c

        lax.fori_loop(0, HKV, body, 0)
        zc[0] += HKV * ZPI
        z_batch(ZB)
        merge_heads(o_scr, l, l)
        return _group_sum(_nn(full_scr[l].astype(bf16), wo_buf[...]))

    def attn_bwd(l, da, last):
        dab = da.astype(bf16)
        split_heads(_nt(dab, wo_buf[...]), do_scr, l)
        lo16_d = (_rows((16, DH)) % 8) < 4

        def body(kv, c):
            z_in_loop(kv)
            dog = do_scr[l, kv]
            dogb = dog.astype(bf16)
            dp = jnp.where(lo_w, _nt(dogb, v_buf[kv]), _nt(dogb, v_buf[HKV + kv]))
            p = p_scr[l, kv]
            ds = p * (dp - jnp.sum(p * dp, axis=-1, keepdims=True)) * SCALE
            dsb = ds.astype(bf16)
            dq_scr[l, kv] = jnp.where(lo_d, _nn(dsb, k_buf[kv]), _nn(dsb, k_buf[HKV + kv]))
            if not last:
                ds_scr[kv] = ds
            else:
                pc = jnp.concatenate([p, p_scr[1 - l, kv]], axis=0).astype(bf16)
                doc = jnp.concatenate([dog, do_scr[1 - l, kv]], axis=0)
                for b in range(NB):
                    sel = lo16_d if b == 0 else jnp.logical_not(lo16_d)
                    v_buf[b * HKV + kv] = _tn(pc, jnp.where(sel, doc, 0.0).astype(bf16)).astype(bf16)
                dsc = jnp.concatenate([ds, ds_scr[kv]], axis=0).astype(bf16)
                qc = jnp.concatenate([q_scr[l, kv], q_scr[1 - l, kv]], axis=0)
                for b in range(NB):
                    sel = lo16_d if b == 0 else jnp.logical_not(lo16_d)
                    k_buf[b * HKV + kv] = _tn(dsc, jnp.where(sel, qc, 0.0).astype(bf16)).astype(bf16)
            return c

        lax.fori_loop(0, HKV, body, 0)
        zc[0] += HKV * ZPI
        z_batch(ZB)
        merge_heads(dq_scr, l, 2 + l)
        return _group_sum(_nt(full_scr[2 + l].astype(bf16), wq_buf[...]))

    def mlp_fwd(nb):
        h = _nn(nb, w1_buf[...]) + b1_ref[...].astype(f32).reshape(1, FF)
        t = jnp.tanh(GELU_C * (h + GELU_A * h * h * h))
        g = 0.5 * h * (1.0 + t)
        gb = g.astype(bf16)
        m = _nn(gb, w2_buf[...]) + b2_ref[...].astype(f32).reshape(1, DM)
        return m, h, t, gb

    def mlp_bwd(dm, h, t):
        dg = _nt(dm.astype(bf16), w2_buf[...])
        gp = 0.5 * (1.0 + t) + 0.5 * h * (1.0 - t * t) * GELU_C * (1.0 + 3.0 * GELU_A * h * h)
        dh = dg * gp
        dn = _nt(dh.astype(bf16), w1_buf[...])
        return dh, dn

    def first_of_group(a):
        return jnp.where(_rows(a.shape) % 4 == 0, a, 0.0)

    for c in s_in:
        c.wait()
    lo_m = _rows((8, DM)) < 4
    xin = x_ref[...].astype(f32)
    x0 = jnp.where(lo_m, xin[0:1, :], xin[1:2, :])
    gin = g_ref[...].astype(f32)
    dx4 = jnp.where(lo_m, gin[0:1, :], gin[1:2, :])

    n1, rs1 = _ln_fwd(x0)
    n1b = n1.astype(bf16)
    x1 = x0 + attn_fwd(0, n1b)
    n2, rs2 = _ln_fwd(x1)
    n2b = n2.astype(bf16)
    m2, h2, t2, g2b = mlp_fwd(n2b)
    x2 = x1 + m2
    n3, rs3 = _ln_fwd(x2)
    n3b = n3.astype(bf16)
    x3 = x2 + attn_fwd(1, n3b)
    n4, rs4 = _ln_fwd(x3)
    n4b = n4.astype(bf16)
    m4, h4, t4, g4b = mlp_fwd(n4b)
    x4 = x3 + m4
    out_ref[...] = jnp.concatenate([x4[0:1, :], x4[4:5, :]], axis=0).astype(out_ref.dtype)
    s_out[0].start()

    dh4, dn4 = mlp_bwd(dx4, h4, t4)
    dx3 = dx4 + _ln_bwd(dn4, n4, rs4)
    dn3 = attn_bwd(1, dx3, False)
    dx2 = dx3 + _ln_bwd(dn3, n3, rs3)
    dh2, dn2 = mlp_bwd(dx2, h2, t2)
    dx1 = dx2 + _ln_bwd(dn2, n2, rs2)

    dm16 = jnp.concatenate([first_of_group(dx2), first_of_group(dx4)], axis=0)
    dh16 = jnp.concatenate([first_of_group(dh2), first_of_group(dh4)], axis=0)
    db2_ref[...] = jnp.sum(dm16, axis=0).astype(db2_ref.dtype)
    db1_ref[...] = jnp.sum(dh16, axis=0).astype(db1_ref.dtype)
    s_out[2].start()
    s_out[3].start()
    g16 = jnp.concatenate([g2b, g4b], axis=0)
    n16m = jnp.concatenate([n2b, n4b], axis=0)
    dw2_buf[...] = _tn(g16, dm16.astype(bf16)).astype(bf16)
    dw1_buf[...] = _tn(n16m, dh16.astype(bf16)).astype(bf16)
    z_batch(ZB)
    o16 = jnp.concatenate([full_scr[0], full_scr[1]], axis=0).astype(bf16)
    da16 = jnp.concatenate([dx1, dx3], axis=0).astype(bf16)
    dwo_buf[...] = _tn(o16, da16).astype(bf16)
    z_batch(ZB)

    dn1 = attn_bwd(0, dx1, True)
    dx0 = dx1 + _ln_bwd(dn1, n1, rs1)
    dx_ref[...] = jnp.concatenate([dx0[0:1, :], dx0[4:5, :]], axis=0).astype(dx_ref.dtype)
    s_out[1].start()

    n16a = jnp.concatenate([n1b, n3b], axis=0)
    dq16 = jnp.concatenate([full_scr[2], full_scr[3]], axis=0).astype(bf16)
    dwq_buf[...] = _tn(n16a, dq16).astype(bf16)

    assert (NR // RG) * NJ == w_ranges[-1][1]
    for lo, hi, which in w_ranges:
        def g_out(i, c, which=which):
            w_chunk(i, which, dw_buf, dw_hbm, wo_sem)
            return win_out(i, c)
        lax.fori_loop(lo, hi, g_out, 0)
    z_batch(NZ - zc[0])

    for c in s_out:
        c.wait()
    for i in range(4):
        pltpu.make_async_copy(dw_buf[i], dw_hbm[i], wo_sem.at[i]).wait()
    for t, (buf, dst) in enumerate(((k_buf, dk_hbm), (v_buf, dv_hbm))):
        zr = dst.at[:, pl.ds(0, NSEG - 1), :, :]
        pltpu.make_async_copy(zr, zr, z_sem.at[t]).wait()
        pltpu.make_async_copy(buf, dst.at[:, NSEG - 1, :, :], o_sem.at[t]).wait()


@jax.jit
def pallas_interleave_layers__sliding_block_cached__dense_activation_gelu__decode_kernel(
    A_x: jax.Array,
    A_k_cache: jax.Array,
    A_v_cache: jax.Array,
    A_wq: jax.Array,
    A_wo: jax.Array,
    B_x: jax.Array,
    B_w1: jax.Array,
    B_b1: jax.Array,
    B_w2: jax.Array,
    B_b2: jax.Array,
    grad_out: jax.Array,
):
    hbm = pl.BlockSpec(memory_space=pl.ANY)
    sds = jax.ShapeDtypeStruct
    out_shape = (
        sds((NB, DM), bf16),
        sds((NB, DM), bf16),
        sds((FF,), bf16),
        sds((DM,), bf16),
        sds((NR, NSEG, WIN, DH), bf16),
        sds((NR, NSEG, WIN, DH), bf16),
        sds((DM, HQ * DH), bf16),
        sds((HQ * DH, DM), bf16),
        sds((DM, FF), bf16),
        sds((FF, DM), bf16),
    )
    scratch = [
        pltpu.VMEM((NB, DM), bf16),
        pltpu.VMEM((NB, DM), bf16),
        pltpu.VMEM((FF,), bf16),
        pltpu.VMEM((DM,), bf16),
        pltpu.VMEM((NB, DM), bf16),
        pltpu.VMEM((NB, DM), bf16),
        pltpu.VMEM((FF,), bf16),
        pltpu.VMEM((DM,), bf16),
        pltpu.VMEM((NR, WIN, DH), bf16),
        pltpu.VMEM((NR, WIN, DH), bf16),
        pltpu.VMEM((DM, HQ * DH), bf16),
        pltpu.VMEM((HQ * DH, DM), bf16),
        pltpu.VMEM((DM, FF), bf16),
        pltpu.VMEM((FF, DM), bf16),
        pltpu.VMEM((RG, ZR, DH), bf16),
        pltpu.VMEM((DM, HQ * DH), bf16),
        pltpu.VMEM((HQ * DH, DM), bf16),
        pltpu.VMEM((DM, FF), bf16),
        pltpu.VMEM((FF, DM), bf16),
        pltpu.VMEM((2, HKV, 8, DH), f32),
        pltpu.VMEM((2, HKV, 8, DH), f32),
        pltpu.VMEM((2, HKV, 8, DH), f32),
        pltpu.VMEM((2, HKV, 8, DH), f32),
        pltpu.VMEM((2, HKV, 8, WIN), f32),
        pltpu.VMEM((HKV, 8, WIN), f32),
        pltpu.VMEM((4, 8, HQ * DH), f32),
        pltpu.SemaphoreType.DMA((2,)),
        pltpu.SemaphoreType.DMA((4,)),
        pltpu.SemaphoreType.DMA((2,)),
        pltpu.SemaphoreType.DMA((2,)),
        pltpu.SemaphoreType.DMA((4,)),
        pltpu.SemaphoreType.DMA((4,)),
        pltpu.SemaphoreType.DMA((4,)),
    ]
    out, dx, db1, db2, dk, dv, dwq, dwo, dw1, dw2 = pl.pallas_call(
        _kernel,
        in_specs=[hbm] * 10,
        out_specs=[hbm] * 10,
        out_shape=out_shape,
        scratch_shapes=scratch,
        compiler_params=pltpu.CompilerParams(vmem_limit_bytes=110 * 1024 * 1024),
    )(A_x.reshape(NB, DM), grad_out.reshape(NB, DM), B_b1, B_b2,
      A_k_cache, A_v_cache, A_wq, A_wo, B_w1, B_w2)
    return (out.reshape(NB, 1, DM), dx.reshape(NB, 1, DM),
            dk.reshape(NB, HKV, SK, DH), dv.reshape(NB, HKV, SK, DH), dwq, dwo, dw1,
            db1, dw2, db2)
```
